```python
import os as _os
_os.environ.setdefault('JAX_PLATFORMS', 'cpu')
import jax
import jax.numpy as jnp

def _softmax(x, axis=-1):
    return jax.nn.softmax(x, axis=axis)

def _gelu(x):
    return jax.nn.gelu(x, approximate=True)

def _silu(x):
    return jax.nn.silu(x)

def _sigmoid(x):
    return jax.nn.sigmoid(x)

def _layernorm(x, axis=-1, eps=1e-05):
    m = jnp.mean(x, axis=axis, keepdims=True)
    v = jnp.var(x, axis=axis, keepdims=True)
    return (x - m) / jnp.sqrt(v + eps)

def _scatter_add(tgt, idx, src, axis=0):
    return tgt.at[idx].add(src)

def _segment_sum(src, seg, n):
    return jax.ops.segment_sum(src, seg, n)

class _Rng:

    def __init__(self, key):
        self._k = key

    def _next(self):
        self._k, sub = jax.random.split(self._k)
        return sub

    def normal(self, shape):
        return jax.random.normal(self._next(), shape, dtype=jnp.bfloat16)

    def randint(self, lo, hi, shape):
        return jax.random.randint(self._next(), shape, lo, hi, dtype=jnp.int32)

    def uniform(self, shape, lo=0.0, hi=1.0):
        return jax.random.uniform(self._next(), shape, jnp.bfloat16, lo, hi)

    def permutation(self, n):
        return jax.random.permutation(self._next(), n)
kernel_name = 'gated_mix__mha_block__memory_aug_recurrent_mem_tr__prompt'

def setup_inputs():
    _rng = _Rng(jax.random.key(int.from_bytes(__import__("os").urandom(4), "little")))
    _w = lambda a: (lambda t: t.astype(jnp.bfloat16) if jnp.issubdtype(t.dtype, jnp.floating) else t)(jnp.asarray(a))

    def _A_setup():
        B, S, D, H = (1, 2048, 512, 32)
        return {'x': _w((lambda *s: _rng.normal(s) * 0.05)(B, S, D)), 'wqkv': _w((lambda *s: _rng.normal(s) * 0.8)(D, 3 * D)), 'wo': _w((lambda *s: _rng.normal(s) * 0.05)(D, D))}
    _A_in = _A_setup()

    def _B_setup():
        B, S, Dm = (1, 2048, 512)
        H, Dh = (32, 128)
        M, seg = (8, 32)
        seg = min(seg, S)
        S = S // seg * seg
        return {'x': _w((lambda *s: _rng.normal(s) * 0.05)(B, S, Dm)), 'mem0': _w((lambda *s: _rng.normal(s) * 0.8)(B, M, Dm)), 'Wq': _w((lambda *s: _rng.normal(s) * 1.6)(Dm, H, Dh) * Dm ** (-0.5)), 'Wk': _w((lambda *s: _rng.normal(s) * 1.6)(Dm, H, Dh) * Dm ** (-0.5)), 'Wv': _w((lambda *s: _rng.normal(s) * 0.8)(Dm, H, Dh) * Dm ** (-0.5)), 'Wo': _w((lambda *s: _rng.normal(s) * 0.8)(H, Dh, Dm) * (H * Dh) ** (-0.5)), 'seg_len': seg}
    _B_in = _B_setup()
    return {'A_x': _A_in['x'], 'A_wqkv': _A_in['wqkv'], 'A_wo': _A_in['wo'], 'B_x': _B_in['x'], 'B_mem0': _B_in['mem0'], 'B_Wq': _B_in['Wq'], 'B_Wk': _B_in['Wk'], 'B_Wv': _B_in['Wv'], 'B_Wo': _B_in['Wo'], 'B_seg_len': _B_in['seg_len'], 'gate_w': _w((lambda *s: _rng.normal(s) * 0.05)(512) * 16.0)}

def reference(A_x, A_wqkv, A_wo, B_x, B_mem0, B_Wq, B_Wk, B_Wv, B_Wo, B_seg_len, gate_w):

    def _A_ref(x, wqkv, wo):
        B, S, D = x.shape
        H = 32
        Dh = D // H
        qkv = (lambda x, *d: x.transpose(*d))((x @ wqkv).reshape(B, S, 3, H, Dh), 2, 0, 3, 1, 4)
        q, k, v = (qkv[0], qkv[1], qkv[2])
        scores = jnp.einsum('bhqd,bhkd->bhqk', q, k) * Dh ** (-0.5)
        p = _softmax(scores, axis=-1)
        o = jnp.einsum('bhqk,bhkd->bhqd', p, v)
        return (lambda x, *d: x.transpose(*d))(o, 0, 2, 1, 3).reshape(B, S, D) @ wo

    def _B_ref(x, mem0, Wq, Wk, Wv, Wo, seg_len):
        B, S, Dm = x.shape
        H, Dh = (Wq.shape[1], Wq.shape[2])
        M = mem0.shape[1]
        scale = Dh ** (-0.5)
        n_seg = S // seg_len
        L = M + seg_len
        idx = jnp.arange(L)
        mask = (idx[:, None] < M) | (idx[:, None] >= idx[None, :])
        mem = mem0
        outs = []
        for s in range(n_seg):
            xs = x[:, s * seg_len:(s + 1) * seg_len, :].copy()
            h = jnp.concatenate([mem, xs], axis=1)
            q = jnp.einsum('btd,dhe->bhte', h, Wq)
            k = jnp.einsum('btd,dhe->bhte', h, Wk)
            v = jnp.einsum('btd,dhe->bhte', h, Wv)
            scores = jnp.einsum('bhqe,bhke->bhqk', q, k) * scale
            scores = jnp.where(mask[None, None], scores, -1000000000.0)
            p = _softmax(scores, axis=-1)
            o = jnp.einsum('bhqk,bhke->bhqe', p, v)
            o = jnp.einsum('bhte,hed->btd', o, Wo)
            mem = o[:, :M, :].copy()
            outs.append(o[:, M:, :])
        return jnp.concatenate(outs, axis=1)
    x = A_x
    g = _sigmoid((x * gate_w).sum(-1, keepdims=True))
    a = _A_ref(x, A_wqkv, A_wo)
    b = _B_ref(x, B_mem0, B_Wq, B_Wk, B_Wv, B_Wo, B_seg_len)
    return g * a + (1 - g) * b
```

```python
import functools
import math

import jax
import jax.numpy as jnp
import jax.experimental.pallas as pl
import jax.experimental.pallas.tpu as pltpu

HA = 32
BQ = 512
BK = 128
LAGC = 1
PLAG = 4
PEEL = 7
XC = 4
NW = 3
RPS = 13
RPARTS = 16
GH = 2
UB = 2
LQ, LV, LW, TV = 1, 3, 8, 2

NT = (((1,), (1,)), ((), ()))
BF = jnp.bfloat16
F32 = jnp.float32
U32 = jnp.uint32
LOG2E = math.log2(math.e)
MASKED = -1e9 * LOG2E
PADDED = -1e30


def _zero_bits(v):
    return (pltpu.bitcast(v, U32) >> 31) >> 1


def _mul_of(v, n):
    return v if isinstance(v, int) else pl.multiple_of(v, n)


def _kernel(seg, H, Dh,
            x_hbm, wqkv_hbm, wo_hbm, mem0_hbm, gw_hbm, wq_hbm, wk_hbm, wv_hbm, woB_hbm,
            out_hbm,
            x_ref, wqkv_ref, wo_ref, mem0_ref, gw_ref, wsrc, wB, woB, qT, kA, vT, oT, oA, obuf,
            sA, sB, sems, osem):
    S, D = x_ref.shape
    M = mem0_ref.shape[0]
    ND = D // 128
    RC = S // XC
    WR = D * H // 2
    DH2 = D // 2

    xcp = [(x_hbm.at[j * RC:(j + 1) * RC], x_ref.at[j * RC:(j + 1) * RC]) for j in range(XC)]
    wcp = [(wqkv_hbm.at[:, j * D:(j + 1) * D], wqkv_ref.at[:, j * D:(j + 1) * D]) for j in range(3)]
    pairs = [wcp[1]] + xcp + [wcp[0], wcp[2]]
    pairs += [(w.bitcast(U32), wsrc.at[i * WR:(i + 1) * WR])
              for i, w in enumerate((wq_hbm, wk_hbm, wv_hbm))]
    pairs += [(woB_hbm.bitcast(U32).at[:, j * 128:(j + 1) * 128], woB.at[j]) for j in range(ND)]
    pairs += [(wo_hbm, wo_ref), (mem0_hbm, mem0_ref), (gw_hbm, gw_ref)]
    cps = [pltpu.make_async_copy(a, b, sems.at[i]) for i, (a, b) in enumerate(pairs)]
    for c in cps:
        c.start()
    cp_wk, cp_wq, cp_wv = cps[0], cps[1 + XC], cps[2 + XC]
    cp_x = cps[1:1 + XC]
    cp_w = cps[3 + XC:6 + XC]
    cp_rest = cps[6 + XC:]

    NREL = 3 * H

    def relayout_piece(gp, z):
        gp = jnp.minimum(gp, NREL * RPARTS - 1)
        i = gp // RPARTS
        part = gp % RPARTS
        w = i // H
        hp = (i % H) // 2
        half = i % 2
        nh = D // 2
        n = nh // RPARTS
        src = wsrc[pl.ds(w * WR + (half * nh + part * n) * (H // 2) + hp, n, stride=H // 2), :]
        src = (src.reshape(n // 8, 8, Dh) | z).reshape(n, Dh)
        lo = pltpu.bitcast(src << 16, F32).astype(BF)
        hi = pltpu.bitcast(src & jnp.uint32(0xFFFF0000), F32).astype(BF)
        r0 = pl.multiple_of((w * H + 2 * hp) * DH2 + half * (nh // 2) + part * (n // 2), n // 2)
        r1 = pl.multiple_of(r0 + DH2, n // 2)
        wB[pl.ds(r0, n // 2), :] = pltpu.bitcast(lo, U32)
        wB[pl.ds(r1, n // 2), :] = pltpu.bitcast(hi, U32)

    dA = D // HA
    dA2 = dA // 2
    hpg = 128 // dA
    qs = (dA ** -0.5) * LOG2E

    def proj_k(j):
        x = x_ref[j * RC:(j + 1) * RC, :]
        kf = jnp.dot(x, wqkv_ref[:, D:2 * D], preferred_element_type=F32).astype(BF)
        for g in range(ND):
            kA[g, j * (RC // 2):(j + 1) * (RC // 2), :] = pltpu.bitcast(
                kf[:, g * 128:(g + 1) * 128], U32)

    def proj_t(wT, dst, j, scale):
        x = x_ref[j * RC:(j + 1) * RC, :]
        r = jax.lax.dot_general(wT, x, NT, preferred_element_type=F32)
        if scale is not None:
            r = r * scale
        dst[:, j * RC:(j + 1) * RC] = pltpu.bitcast(r.astype(BF), U32)

    cp_wk.wait()
    for j in range(NW):
        cp_x[j].wait()
        proj_k(j)
    for c in cp_x[NW:] + [cp_wq, cp_wv]:
        c.wait()
    for j in range(NW, XC):
        proj_k(j)
    wqT = wqkv_ref[:, 0:D].astype(F32).T.astype(BF)
    wvT = wqkv_ref[:, 2 * D:].astype(F32).T.astype(BF)
    for j in range(XC):
        proj_t(wqT, qT, j, qs)
        proj_t(wvT, vT, j, None)

    nqb = S // BQ
    NI = HA * nqb
    NC = S // BK

    def idx(it):
        blk, j = it
        g = blk // nqb
        q0 = _mul_of((blk % nqb) * BQ, BQ)
        h2 = _mul_of((g * hpg + j) * dA2, dA2)
        return q0, g, h2, j

    def item(t, u):
        return (t + u // hpg, u % hpg)

    def pv_chunk(sref, c, m, h2, l, o):
        ks = slice(c * BK, (c + 1) * BK)
        p = jnp.exp2(sref[ks, :].reshape(BK // 8, 8, BQ) - m)
        acc = l
        for r in reversed(range(BK // 8)):
            acc = p[r] if acc is None else acc + p[r]
        v = vT[pl.ds(h2, dA2), ks]
        if l is not None:
            lb = pltpu.bitcast(l, U32)
            z = lb[:, 0:128]
            for t in range(1, BQ // 128):
                z = z | lb[:, t * 128:(t + 1) * 128]
            v = v | ((z >> 31) >> 1)
        pv = jnp.dot(pltpu.bitcast(v, BF), p.reshape(BK, BQ).astype(BF),
                     preferred_element_type=F32)
        return acc, (pv if o is None else o + pv)

    def finalize(it, l, o):
        p0, g, _, j = idx(it)
        lt = jnp.sum(l, axis=0, keepdims=True)
        oT[j * dA:(j + 1) * dA, :] = o / lt
        if j == hpg - 1:
            oA[g, pl.ds(_mul_of(p0 // 2, BQ // 2), BQ // 2), :] = pltpu.bitcast(
                oT[...].T.astype(BF), U32)

    def stage(i1, s1, i2, s2, m2, tail, rel=None):
        if i1 is not None:
            q0, g1, h2, j = idx(i1)
            qh = qT[pl.ds(h2, dA2), pl.ds(q0, BQ)]
            parts = [jnp.zeros((dA2 * j, BQ), U32), qh, jnp.zeros((dA2 * (hpg - 1 - j), BQ), U32)]
            qp = pltpu.bitcast(jnp.concatenate([p for p in parts if p.shape[0]], axis=0), BF)
        if i2 is not None:
            hv = idx(i2)[2]
        l = o = mx = None
        mcs = []

        def pin(m, c):
            if len(mcs) > c - PLAG >= 0:
                return pltpu.bitcast(pltpu.bitcast(m, U32) | _zero_bits(mcs[c - PLAG]), F32)
            return m

        for c in range(NC):
            if i1 is not None:
                kc = pltpu.bitcast(kA[g1, c * (BK // 2):(c + 1) * (BK // 2), :], BF)
                sv = jnp.dot(kc, qp, preferred_element_type=F32)
                s1[c * BK:(c + 1) * BK, :] = sv
                sv3 = sv.reshape(BK // 8, 8, BQ)
                mc = sv3[0]
                for r_ in range(1, BK // 8):
                    mc = jnp.maximum(mc, sv3[r_])
                mx = mc if c == 0 else jnp.maximum(mx, mc)
                mcs.append(mc)
                if rel is not None and c < RPS:
                    relayout_piece(rel * RPS + c, _zero_bits(mc[:, 0:128]))
            if c < LAGC:
                if tail is not None:
                    ti, tb, tm, tl, to = tail
                    tl, to = pv_chunk(tb, NC - LAGC + c, pin(tm, c), idx(ti)[2], tl, to)
                    tail[3], tail[4] = tl, to
                    if c == LAGC - 1:
                        finalize(ti, tl, to)
            elif i2 is not None:
                l, o = pv_chunk(s2, c - LAGC, pin(m2, c), hv, l, o)
        m1 = None
        if i1 is not None:
            m1 = jnp.broadcast_to(jnp.max(mx, axis=0, keepdims=True), (8, BQ))
        return m1, ((m2, l, o) if i2 is not None else None)

    def run_stage(t, u, carry, first=False, last=False, rel=None):
        a, b = (sA, sB) if u % 2 == 0 else (sB, sA)
        m, tl = carry
        tail = None if first else [item(t - 1, u - 1 + hpg), b, tl[0], tl[1], tl[2]]
        return stage(None if last else item(t, u + 1), b, item(t, u), a, m, tail, rel)

    assert RPS <= NC and PEEL % 2 == 1 and hpg % 2 == 0
    m0, _ = stage(item(0, 0), sA, None, None, None, None)
    carry = run_stage(0, 0, (m0, None), first=True)
    for u in range(1, PEEL):
        carry = run_stage(0, u, carry)

    for c in cp_w:
        c.wait()

    def loop_a(t, carry):
        for u in range(PEEL, PEEL + hpg):
            carry = run_stage(t, u, carry, rel=t * hpg + (u - PEEL))
        return carry

    nit = (NI - 1 - PEEL) // hpg
    assert nit * hpg * RPS >= NREL * RPARTS
    carry = jax.lax.fori_loop(0, nit, loop_a, carry)
    for i in range(nit * hpg + PEEL, NI):
        carry = run_stage(nit, i - nit * hpg, carry, last=(i == NI - 1))
    tm, tl, to = carry[1]
    last_item = item(nit, NI - 1 - nit * hpg)
    for c in range(NC - LAGC, NC):
        tl, to = pv_chunk(sA if (NI - 1) % 2 == 0 else sB, c, tm, idx(last_item)[2], tl, to)
    finalize(last_item, tl, to)

    for c in cp_rest:
        c.wait()
    L = M + seg
    X = -(-L // 16) * 16 - L
    assert (L - X) % 16 == 0 and X % 8 == 0 and M % 8 == 0
    R = GH * L
    RP = -(-R // 128) * 128
    assert R % 16 == 0
    sc = (Dh ** -0.5) * LOG2E
    ri = jax.lax.broadcasted_iota(jnp.int32, (R, RP), 0)
    ci = jax.lax.broadcasted_iota(jnp.int32, (R, RP), 1)
    same = ci < R
    rl, cl = ri, ci
    for a in range(1, GH):
        same = same & ((ri >= a * L) == (ci >= a * L))
        rl = jnp.where(ri >= a * L, ri - a * L, rl)
        cl = jnp.where(ci >= a * L, ci - a * L, cl)
    vis = same & ((rl < M) | (rl >= cl))
    fill = jnp.where(same, MASKED, PADDED).astype(F32)
    kpad = jnp.zeros((RP - R, Dh), F32)

    def proj(hh, h):
        wsl = lambda w: pltpu.bitcast(wB[(w * H + h) * DH2:(w * H + h + 1) * DH2, :], BF)
        q = jnp.dot(hh, wsl(0), preferred_element_type=F32) * sc
        k = jnp.dot(hh, wsl(1), preferred_element_type=F32)
        v = jnp.dot(hh, wsl(2), preferred_element_type=F32)
        return q, k, v

    def attn_qk(qs_, ks_):
        q2 = jnp.concatenate(qs_, axis=0).astype(BF)
        k2 = jnp.concatenate(ks_ + [kpad], axis=0).astype(BF)
        s = jax.lax.dot_general(q2, k2, NT, preferred_element_type=F32)
        s = jnp.where(vis, s, fill)
        p = jnp.exp2(s - jnp.max(s, axis=-1, keepdims=True))
        l = jnp.sum(p, axis=-1, keepdims=True)
        r = pl.reciprocal(l, approx=True)
        r = r * (2.0 - l * r)
        return p.astype(BF), r

    def attn_pv(p, r, vs_):
        v2 = jnp.concatenate(vs_ + [kpad], axis=0).astype(BF)
        o = jnp.dot(p, v2, preferred_element_type=F32) * r
        return [o[a * L:(a + 1) * L] for a in range(GH)]

    def wo_part(o_rows, h):
        w = jnp.concatenate(
            [pltpu.bitcast(woB[j, h * (Dh // 2):(h + 1) * (Dh // 2), :], BF) for j in range(ND)],
            axis=1)
        return jnp.dot(o_rows.astype(BF), w, preferred_element_type=F32)

    NG = H // GH
    sched = []
    for g in range(NG):
        sched.append(('P', g))
        if g - LV >= 0:
            sched.append(('V', g - LV))
        if g - LQ >= 0:
            sched.append(('Q', g - LQ))
        if g - LW >= 0:
            sched.append(('W', g - LW))
    tw = [('W', g) for g in range(NG - LW, NG)]
    for g in range(NG, NG + LV):
        sched.append(('V', g - LV))
        if g - LQ < NG:
            sched.append(('Q', g - LQ))
        n = TV if g < NG + LV - 1 else 0
        n = min(n, len([w for w in tw if w[1] <= g - LV]))
        sched += tw[:n]
        tw = tw[n:]
    sched += tw

    def step(hh, pick, wo_rows):
        y = None
        qkv, pr, outs = {}, {}, {}
        for kind, g in sched:
            if kind == 'P':
                qkv[g] = [pick(h, *proj(hh, h)) for h in range(g * GH, (g + 1) * GH)]
            elif kind == 'Q':
                pr[g] = attn_qk([a[0] for a in qkv[g]], [a[1] for a in qkv[g]])
            elif kind == 'V':
                p, r = pr.pop(g)
                for a, o in enumerate(attn_pv(p, r, [a[2] for a in qkv[g]])):
                    outs[g * GH + a] = o
            else:
                for h in range(g * GH, (g + 1) * GH):
                    part = wo_part(wo_rows(h, outs[h]), h)
                    y = part if y is None else y + part
        return y, outs

    gw = gw_ref[...].astype(F32).reshape(1, D)

    def a_rows(r, n):
        r2 = pl.multiple_of(r // 2, n // 2)
        oa = jnp.concatenate(
            [pltpu.bitcast(oA[g, pl.ds(r2, n // 2), :], BF) for g in range(ND)], axis=1)
        return jnp.dot(oa, wo_ref[...], preferred_element_type=F32)

    def pair(r0, mem):
        xf = x_ref[pl.ds(r0, 2 * seg), :].astype(F32)
        keep = {}

        def pick0(h, q, k, v):
            keep[h] = (q[L:], k[L:], v[L:])
            return q[0:L], k[0:L], v[0:L]

        def pick1(h, q, k, v):
            cat = lambda a0, a1: jnp.concatenate([a1[0:M], a0, a1[M:]], axis=0)
            return tuple(cat(a0, a1) for a0, a1 in zip(keep[h], (q, k, v)))

        h0 = jnp.concatenate([mem, xf[0:seg + X]], axis=0).astype(BF)
        y0, o0 = step(h0, pick0, lambda h, o: o[0:L - X])
        a0 = a_rows(r0, seg)
        h1 = jnp.concatenate([y0[0:M], xf[seg + X:]], axis=0).astype(BF)
        y1, _ = step(h1, pick1,
                     lambda h, o: jnp.concatenate([o[0:M], o0[h][L - X:L], o[M:L]], axis=0))
        a1 = a_rows(r0 + seg, seg)
        b = jnp.concatenate([y0[M:], y1[M:]], axis=0)
        a = jnp.concatenate([a0, a1], axis=0)
        g = jax.nn.sigmoid(jnp.sum(xf * gw, axis=-1, keepdims=True))
        obuf[pl.ds(r0, 2 * seg), :] = (g * a + (1 - g) * b).astype(obuf.dtype)
        return y1[0:M].astype(BF).astype(F32)

    RI = UB * 2 * seg
    NP = S // RI

    def out_copy(t):
        r = _mul_of(t * RI, RI)
        return pltpu.make_async_copy(obuf.at[pl.ds(r, RI), :], out_hbm.at[pl.ds(r, RI), :], osem)

    def loop_b(t, mem):
        for u in range(UB):
            mem = pair(pl.multiple_of(t * RI + u * 2 * seg, 2 * seg), mem)
        out_copy(t).start()
        return mem

    jax.lax.fori_loop(0, NP, loop_b, mem0_ref[...].astype(F32))
    for t in range(NP):
        out_copy(t).wait()


def pallas_gated_mix__mha_block__memory_aug_recurrent_mem_tr__prompt_kernel(
        A_x, A_wqkv, A_wo, B_x, B_mem0, B_Wq, B_Wk, B_Wv, B_Wo, B_seg_len, gate_w):
    del B_x
    seg = int(B_seg_len)
    B, S, D = A_x.shape
    _, H, Dh = B_Wq.shape
    M = B_mem0.shape[1]
    E = H * Dh
    ND = D // 128
    assert B == 1 and Dh == 128 and S % (UB * 2 * seg) == 0 and S % BQ == 0
    hbm = pl.BlockSpec(memory_space=pltpu.HBM)
    out = pl.pallas_call(
        functools.partial(_kernel, seg, H, Dh),
        out_shape=jax.ShapeDtypeStruct((S, D), A_x.dtype),
        in_specs=[hbm] * 9,
        out_specs=hbm,
        scratch_shapes=[
            pltpu.VMEM((S, D), BF), pltpu.VMEM((D, 3 * D), BF), pltpu.VMEM((D, D), BF),
            pltpu.VMEM((M, D), BF), pltpu.VMEM((D,), BF),
            pltpu.VMEM((3 * D * H // 2 + H // 2, Dh), U32),
            pltpu.VMEM((3 * H * D // 2, Dh), U32),
            pltpu.VMEM((ND, E // 2, 128), U32),
            pltpu.VMEM((D // 2, S), U32),
            pltpu.VMEM((ND, S // 2, 128), U32),
            pltpu.VMEM((D // 2, S), U32),
            pltpu.VMEM((128, BQ), F32),
            pltpu.VMEM((ND, S // 2, 128), U32),
            pltpu.VMEM((S, D), A_x.dtype),
            pltpu.VMEM((S, BQ), F32), pltpu.VMEM((S, BQ), F32),
            pltpu.SemaphoreType.DMA((9 + XC + ND,)), pltpu.SemaphoreType.DMA(()),
        ],
        compiler_params=pltpu.CompilerParams(vmem_limit_bytes=100 * 1024 * 1024),
    )(A_x.reshape(S, D), A_wqkv, A_wo, B_mem0.reshape(M, D), gate_w,
      B_Wq.reshape(D * H, Dh), B_Wk.reshape(D * H, Dh), B_Wv.reshape(D * H, Dh),
      B_Wo.reshape(E, D))
    return out.reshape(B, S, D)
```
